```python
import os as _os
_os.environ.setdefault('JAX_PLATFORMS', 'cpu')
import jax
import jax.numpy as jnp

def _softmax(x, axis=-1):
    return jax.nn.softmax(x, axis=axis)

def _gelu(x):
    return jax.nn.gelu(x, approximate=True)

def _silu(x):
    return jax.nn.silu(x)

def _sigmoid(x):
    return jax.nn.sigmoid(x)

def _layernorm(x, axis=-1, eps=1e-05):
    m = jnp.mean(x, axis=axis, keepdims=True)
    v = jnp.var(x, axis=axis, keepdims=True)
    return (x - m) / jnp.sqrt(v + eps)

def _scatter_add(tgt, idx, src, axis=0):
    return tgt.at[idx].add(src)

def _segment_sum(src, seg, n):
    return jax.ops.segment_sum(src, seg, n)

class _Rng:

    def __init__(self, key):
        self._k = key

    def _next(self):
        self._k, sub = jax.random.split(self._k)
        return sub

    def normal(self, shape):
        return jax.random.normal(self._next(), shape, dtype=jnp.bfloat16)

    def randint(self, lo, hi, shape):
        return jax.random.randint(self._next(), shape, lo, hi, dtype=jnp.int32)

    def uniform(self, shape, lo=0.0, hi=1.0):
        return jax.random.uniform(self._next(), shape, jnp.bfloat16, lo, hi)

    def permutation(self, n):
        return jax.random.permutation(self._next(), n)
kernel_name = 'adaLN_cond__sliding_local_dilated__dense_activation_relu__prompt'

def setup_inputs():
    _rng = _Rng(jax.random.key(int.from_bytes(__import__("os").urandom(4), "little")))
    _w = lambda a: (lambda t: t.astype(jnp.bfloat16) if jnp.issubdtype(t.dtype, jnp.floating) else t)(jnp.asarray(a))

    def _A_setup():
        B, S, D = (1, 2048, 576)
        return {'x': _w((lambda *s: _rng.normal(s) * 0.05)(B, S, D)), 'wqkv': _w((lambda *s: _rng.normal(s) * 0.05)(D, 3 * D)), 'wo': _w((lambda *s: _rng.normal(s) * 0.05)(D, D))}
    _A_in = _A_setup()

    def _B_setup():
        B, S, D, Dff = (1, 2048, 576, 4608)
        return {'x': _w((lambda *s: _rng.normal(s) * 0.05)(B, S, D)), 'w1': _w((lambda *s: _rng.normal(s) * 0.05)(D, Dff)), 'w2': _w((lambda *s: _rng.normal(s) * 0.05)(Dff, D))}
    _B_in = _B_setup()
    return {'A_x': _A_in['x'], 'A_wqkv': _A_in['wqkv'], 'A_wo': _A_in['wo'], 'B_x': _B_in['x'], 'B_w1': _B_in['w1'], 'B_w2': _B_in['w2'], 'c': _w((lambda *s: _rng.normal(s) * 0.05)(1, 576) * 8.0), 'w_mod': _w((lambda *s: _rng.normal(s) * 0.05)(576, 6 * 576) * 576 ** (-0.5) * 8.0)}

def reference(A_x, A_wqkv, A_wo, B_x, B_w1, B_w2, c, w_mod):

    def _A_ref(x, wqkv, wo):
        B, S, D = x.shape
        H = 32
        Dh = D // H
        W, dil = (8, 2)
        qkv = (lambda x, *d: x.transpose(*d))((x @ wqkv).reshape(B, S, 3, H, Dh), 2, 0, 3, 1, 4)
        q, k, v = (qkv[0], qkv[1], qkv[2])
        scale = Dh ** (-0.5)
        pos = jnp.arange(S)
        off = jnp.arange(W) * dil
        idx = pos[:, None] - off[None, :]
        mask = idx >= 0
        idx_c = jnp.where(mask, idx, 0).reshape(-1)
        kg = k[:, :, idx_c, :].reshape(B, H, S, W, Dh)
        vg = v[:, :, idx_c, :].reshape(B, H, S, W, Dh)
        logits = jnp.einsum('bhsd,bhswd->bhsw', q, kg) * scale
        logits = jnp.where(mask[None, None, :, :], logits, -1000000000.0)
        attn = _softmax(logits, axis=-1)
        o = jnp.einsum('bhsw,bhswd->bhsd', attn, vg)
        return (lambda x, *d: x.transpose(*d))(o, 0, 2, 1, 3).reshape(B, S, D) @ wo

    def _B_ref(x, w1, w2):
        h = jnp.einsum('bsd,df->bsf', x, w1)
        zero = jnp.zeros_like(h)
        h = jnp.maximum(h, zero)
        return jnp.einsum('bsf,fd->bsd', h, w2)
    x = A_x
    mod = (_silu(c) @ w_mod).reshape(c.shape[0], 6, 1, -1)
    sa, ca, ga, sb, cb, gb = (mod[:, 0].copy(), mod[:, 1].copy(), mod[:, 2].copy(), mod[:, 3].copy(), mod[:, 4].copy(), mod[:, 5].copy())
    h = _layernorm(x, axis=-1) * (1 + ca) + sa
    x = x + ga * _A_ref(h, A_wqkv, A_wo)
    h = _layernorm(x, axis=-1) * (1 + cb) + sb
    x = x + gb * _B_ref(h, B_w1, B_w2)
    return x
```

```python
import jax
import jax.numpy as jnp
import jax.experimental.pallas as pl
import jax.experimental.pallas.tpu as pltpu

S = 2048
D = 576
H = 32
DH = 18
W = 8
DIL = 2
DFF = 4608
T = 256
NB = S // T
NC = T // 128
FC = 1152
EPS = 1e-5
NEG = -1000000000.0
SCALE = DH ** (-0.5)

_NT = (((1,), (1,)), ((), ()))


def _layernorm_t(x):
    mu = jnp.mean(x, axis=0, keepdims=True)
    xc = x - mu
    var = jnp.mean(xc * xc, axis=0, keepdims=True)
    return xc * jax.lax.rsqrt(var + EPS)


def _kernel(x_ref, c_ref, wqkv_hbm, wo_hbm, w1_hbm, w2t_hbm, wmod_hbm, o_ref,
            wqkv_v, wo_v, w1_v, w2t_v, wmod_v, wqkv_p, wo_p, mod_v,
            q_s, kbuf, vbuf, o_s, h2_s, x1_s, sems):
    i = pl.program_id(0)

    cp_qkv = pltpu.make_async_copy(wqkv_hbm, wqkv_v, sems.at[0])
    cp_wo = pltpu.make_async_copy(wo_hbm, wo_v, sems.at[1])
    cp_mod = pltpu.make_async_copy(wmod_hbm, wmod_v, sems.at[2])
    cp_w1 = pltpu.make_async_copy(w1_hbm, w1_v, sems.at[3])
    cp_w2 = pltpu.make_async_copy(w2t_hbm, w2t_v, sems.at[4])

    def prologue():
        cp_qkv.start()
        cp_wo.start()
        cp_mod.start()
        cp_w1.start()
        cp_w2.start()
        kbuf[:, 0:128] = jnp.zeros((D, 128), jnp.float32)
        vbuf[:, 0:128] = jnp.zeros((D, 128), jnp.float32)

        a0 = jax.lax.broadcasted_iota(jnp.int32, (D, D), 0)
        a1 = jax.lax.broadcasted_iota(jnp.int32, (D, D), 1)
        perm_t = jnp.where(a1 == (a0 & 31) * DH + (a0 >> 5), 1.0, 0.0).astype(jnp.bfloat16)
        perm = jnp.where(a0 == (a1 & 31) * DH + (a1 >> 5), 1.0, 0.0).astype(jnp.bfloat16)

        cp_qkv.wait()
        for t in range(3):
            wqkv_p[t * D:(t + 1) * D, :] = jax.lax.dot_general(
                perm_t, wqkv_v[:, t * D:(t + 1) * D], _NT,
                preferred_element_type=jnp.float32).astype(jnp.bfloat16)
        cp_wo.wait()
        wo_t = wo_v[...].astype(jnp.float32).T.astype(jnp.bfloat16)
        wo_p[...] = jnp.dot(wo_t, perm,
                            preferred_element_type=jnp.float32).astype(jnp.bfloat16)

        cp_mod.wait()
        cf = c_ref[...].astype(jnp.float32)
        sc = (cf * jax.nn.sigmoid(cf)).astype(jnp.bfloat16)
        scb = jnp.broadcast_to(sc, (128, D))
        mod = jnp.dot(scb, wmod_v[...], preferred_element_type=jnp.float32)
        for t in range(6):
            mod_v[t] = mod[:, t * D:(t + 1) * D].T

    def col(t):
        m = mod_v[t]
        return jnp.concatenate([m] * NC, axis=1) if NC > 1 else m

    lane = jax.lax.broadcasted_iota(jnp.int32, (H, 128), 1)

    def shifted(buf, r0, c, w):
        cur = buf[r0:r0 + H, (c + 1) * 128:(c + 2) * 128]
        if w == 0:
            return cur
        prev = buf[r0:r0 + H, c * 128:(c + 1) * 128]
        z = jnp.where(lane >= 128 - DIL * w, prev, cur)
        return pltpu.roll(z, DIL * w, 1)

    def a_qkv():
        x = x_ref[...].astype(jnp.float32)
        h = (_layernorm_t(x) * (1.0 + col(1)) + col(0)).astype(jnp.bfloat16)
        qkv = jnp.dot(wqkv_p[...], h, preferred_element_type=jnp.float32)
        q_s[...] = qkv[0:D, :] * SCALE
        kbuf[:, 128:128 + T] = qkv[D:2 * D, :]
        vbuf[:, 128:128 + T] = qkv[2 * D:3 * D, :]

    def a_attn(c):
        pos = i * T + c * 128 + lane
        logits = [None] * W
        for d in range(DH):
            qd = q_s[d * H:(d + 1) * H, c * 128:(c + 1) * 128]
            for w in range(W):
                t = qd * shifted(kbuf, d * H, c, w)
                logits[w] = t if logits[w] is None else logits[w] + t
        logits = [jnp.where(pos >= DIL * w, logits[w], NEG) for w in range(W)]
        m = logits[0]
        for w in range(1, W):
            m = jnp.maximum(m, logits[w])
        es = [jnp.exp(l - m) for l in logits]
        den = es[0]
        for w in range(1, W):
            den = den + es[w]
        inv = 1.0 / den
        ps = [e * inv for e in es]
        for d in range(DH):
            acc = None
            for w in range(W):
                t = ps[w] * shifted(vbuf, d * H, c, w)
                acc = t if acc is None else acc + t
            o_s[d * H:(d + 1) * H, c * 128:(c + 1) * 128] = acc.astype(jnp.bfloat16)

    def a_out(slot):
        kbuf[:, 0:128] = kbuf[:, T:T + 128]
        vbuf[:, 0:128] = vbuf[:, T:T + 128]
        a = jnp.dot(wo_p[...], o_s[...], preferred_element_type=jnp.float32)
        x1 = x_ref[...].astype(jnp.float32) + col(2) * a
        x1_s[slot] = x1
        h2t = _layernorm_t(x1) * (1.0 + col(4)) + col(3)
        h2_s[slot] = h2t.T.astype(jnp.bfloat16)

    def part_a(slot):
        a_qkv()
        for c in range(NC):
            a_attn(c)
        a_out(slot)

    def ffn_chunk_static(slot, cidx):
        hc = jnp.dot(h2_s[slot], w1_v[:, cidx * FC:(cidx + 1) * FC],
                     preferred_element_type=jnp.float32)
        hc = jnp.maximum(hc, 0.0).astype(jnp.bfloat16)
        return jax.lax.dot_general(w2t_v[:, cidx * FC:(cidx + 1) * FC], hc, _NT,
                                   preferred_element_type=jnp.float32)

    def steady(cur, prv):
        f = ffn_chunk_static(prv, 0)
        a_qkv()
        f = f + ffn_chunk_static(prv, 1)
        a_attn(0)
        f = f + ffn_chunk_static(prv, 2)
        a_attn(1)
        f = f + ffn_chunk_static(prv, 3)
        o_ref[...] = (x1_s[prv] + col(5) * f).astype(o_ref.dtype)
        a_out(cur)

    def part_b(slot):
        h2 = h2_s[slot]
        f = None
        for cidx in range(DFF // FC):
            hc = jnp.dot(h2, w1_v[:, cidx * FC:(cidx + 1) * FC],
                         preferred_element_type=jnp.float32)
            hc = jnp.maximum(hc, 0.0).astype(jnp.bfloat16)
            part = jax.lax.dot_general(w2t_v[:, cidx * FC:(cidx + 1) * FC], hc, _NT,
                                       preferred_element_type=jnp.float32)
            f = part if f is None else f + part
        o_ref[...] = (x1_s[slot] + col(5) * f).astype(o_ref.dtype)

    def part_b_loop(slot):
        h2 = h2_s[slot]

        def ffn_chunk(cidx, f):
            off = pl.multiple_of(cidx * FC, 128)
            hc = jnp.dot(h2, w1_v[:, pl.ds(off, FC)],
                         preferred_element_type=jnp.float32)
            hc = jnp.maximum(hc, 0.0).astype(jnp.bfloat16)
            part = jax.lax.dot_general(w2t_v[:, pl.ds(off, FC)], hc, _NT,
                                       preferred_element_type=jnp.float32)
            return f + part
        f = jax.lax.fori_loop(0, DFF // FC, ffn_chunk, jnp.zeros((D, T), jnp.float32))
        o_ref[...] = (x1_s[slot] + col(5) * f).astype(o_ref.dtype)

    cur = i % 2
    prv = 1 - cur

    @pl.when(i == 0)
    def _first():
        prologue()
        part_a(0)
        cp_w1.wait()
        cp_w2.wait()

    @pl.when(jnp.logical_and(i > 0, i < NB))
    def _steady():
        steady(cur, prv)

    @pl.when(i == NB)
    def _last():
        part_b_loop(prv)


@jax.jit
def pallas_adaLN_cond__sliding_local_dilated__dense_activation_relu__prompt_kernel(
    A_x: jax.Array,
    A_wqkv: jax.Array,
    A_wo: jax.Array,
    B_x: jax.Array,
    B_w1: jax.Array,
    B_w2: jax.Array,
    c: jax.Array,
    w_mod: jax.Array,
):
    xt = A_x.reshape(S, D).T
    w2t = B_w2.T
    hbm_spec = pl.BlockSpec(memory_space=pltpu.MemorySpace.HBM)
    out_t = pl.pallas_call(
        _kernel,
        grid=(NB + 1,),
        in_specs=[
            pl.BlockSpec((D, T), lambda i: (0, jnp.minimum(i, NB - 1))),
            pl.BlockSpec((1, D), lambda i: (0, 0)),
            hbm_spec, hbm_spec, hbm_spec, hbm_spec, hbm_spec,
        ],
        out_specs=pl.BlockSpec((D, T), lambda i: (0, jnp.maximum(i - 1, 0))),
        out_shape=jax.ShapeDtypeStruct((D, S), jnp.bfloat16),
        scratch_shapes=[
            pltpu.VMEM((D, 3 * D), jnp.bfloat16),
            pltpu.VMEM((D, D), jnp.bfloat16),
            pltpu.VMEM((D, DFF), jnp.bfloat16),
            pltpu.VMEM((D, DFF), jnp.bfloat16),
            pltpu.VMEM((D, 6 * D), jnp.bfloat16),
            pltpu.VMEM((3 * D, D), jnp.bfloat16),
            pltpu.VMEM((D, D), jnp.bfloat16),
            pltpu.VMEM((6, D, 128), jnp.float32),
            pltpu.VMEM((D, T), jnp.float32),
            pltpu.VMEM((D, T + 128), jnp.float32),
            pltpu.VMEM((D, T + 128), jnp.float32),
            pltpu.VMEM((D, T), jnp.bfloat16),
            pltpu.VMEM((2, T, D), jnp.bfloat16),
            pltpu.VMEM((2, D, T), jnp.float32),
            pltpu.SemaphoreType.DMA((5,)),
        ],
        compiler_params=pltpu.CompilerParams(
            dimension_semantics=("arbitrary",),
            vmem_limit_bytes=100 * 1024 * 1024,
        ),
    )(xt, c, A_wqkv, A_wo, B_w1, w2t, w_mod)
    return out_t.T.reshape(1, S, D)
```
